```python
import os as _os
_os.environ.setdefault("JAX_PLATFORMS", "cpu")
import jax
import jax.numpy as jnp

def _softmax(x, axis=-1):
    return jax.nn.softmax(x, axis=axis)
def _gelu(x):
    return jax.nn.gelu(x, approximate=True)
def _silu(x):
    return jax.nn.silu(x)
def _sigmoid(x):
    return jax.nn.sigmoid(x)
def _layernorm(x, axis=-1, eps=1e-5):
    m = jnp.mean(x, axis=axis, keepdims=True)
    v = jnp.var(x, axis=axis, keepdims=True)
    return (x - m) / jnp.sqrt(v + eps)
def _scatter_add(tgt, idx, src, axis=0):
    return tgt.at[idx].add(src)
def _segment_sum(src, seg, n):
    return jax.ops.segment_sum(src, seg, n)
class _Rng:
    def __init__(self, key):
        self._k = key
    def _next(self):
        self._k, sub = jax.random.split(self._k)
        return sub
    def normal(self, shape):
        return jax.random.normal(self._next(), shape, dtype=jnp.bfloat16)
    def randint(self, lo, hi, shape):
        return jax.random.randint(self._next(), shape, lo, hi, dtype=jnp.int32)
    def uniform(self, shape, lo=0.0, hi=1.0):
        return jax.random.uniform(self._next(), shape, jnp.bfloat16, lo, hi)
    def permutation(self, n):
        return jax.random.permutation(self._next(), n)


kernel_name = 'standalone__sliding_local_fixed_window__prompt'

def setup_inputs():
    _rng = _Rng(jax.random.key(int.from_bytes(__import__("os").urandom(4), "little")))
    _w = (lambda a: (lambda t: t.astype(jnp.bfloat16) if jnp.issubdtype(t.dtype, jnp.floating) else t)(jnp.asarray(a)))
    B, H, S, D = 1, 32, 2048, 128
    return {
        "q": _w((lambda *s: _rng.normal(s) * 0.4)(B, H, S, D)),
        "k": _w((lambda *s: _rng.normal(s) * 0.4)(B, H, S, D)),
        "v": _w((lambda *s: _rng.normal(s) * 0.05)(B, H, S, D)),
    }

def reference(q, k, v):
    B, H, S, D = q.shape
    w = 32
    pos = jnp.arange(S)
    rel = pos[:, None] - pos[None, :]
    mask = (rel >= 0) & (rel < w)
    scores = jnp.einsum("bhqd,bhkd->bhqk", q, k) * (D ** -0.5)
    scores = jnp.where(mask[None, None], scores, (lambda x, dt: x.astype(dt))(jnp.array(-1e9), q.dtype))
    p = _softmax(scores, axis=-1)
    return jnp.einsum("bhqk,bhkd->bhqd", p, v)
```

```python
import jax
import jax.numpy as jnp
import numpy as np
from jax import lax
import jax.experimental.pallas as pl
import jax.experimental.pallas.tpu as pltpu

_WINDOW = 32
_MASK_VALUE = -1e9
_TILE = 128
_QBLK = _TILE - _WINDOW
_READ_CHUNKS = (8, 8, 8, 4, 4)
_READ_TAIL = 512
_WRITE_ROWS = 128
_DENSE_ROWS = 16


def _dot_nt(a, b):
    return lax.dot_general(
        a, b, (((1,), (1,)), ((), ())), preferred_element_type=jnp.float32
    )


def _banded_head(q_ref, k_ref, v_ref, o_ref):
    seq, dim = q_ref.shape
    c = float(dim**-0.5 * np.log2(np.e))

    def block(q0, rows, k0, mask):
        s = _dot_nt(q_ref[q0 : q0 + rows, :], k_ref[k0 : k0 + _TILE, :])
        s = jnp.where(mask, s, -jnp.inf)
        m = jnp.max(s, axis=1, keepdims=True)
        p = jnp.exp2((s - m) * c)
        l = jnp.sum(p, axis=1, keepdims=True)
        o = jnp.dot(
            p.astype(v_ref.dtype),
            v_ref[k0 : k0 + _TILE, :],
            preferred_element_type=jnp.float32,
        )
        o_ref[q0 : q0 + rows, :] = (o / l).astype(o_ref.dtype)
        return m

    def band(rows, shift):
        rel = (
            lax.broadcasted_iota(jnp.int32, (rows, _TILE), 0)
            - lax.broadcasted_iota(jnp.int32, (rows, _TILE), 1)
            + shift
        )
        return (rel >= 0) & (rel < _WINDOW)

    first = block(0, _TILE, 0, band(_TILE, 0))
    mask = band(_QBLK, _WINDOW)
    low = None
    for q0 in range(_TILE, seq, _QBLK):
        m = block(q0, _QBLK, q0 - _WINDOW, mask)
        low = m if low is None else jnp.minimum(low, m)
    return jnp.minimum(jnp.min(first), jnp.min(low))


def _dense_head(q_ref, k_ref, v_ref, o_ref):
    seq, dim = q_ref.shape
    dt = q_ref.dtype
    scale = float(np.asarray(dim**-0.5, dtype=dt))
    masked = float(np.asarray(_MASK_VALUE, dtype=dt))

    @pl.loop(0, seq // _DENSE_ROWS)
    def _(i):
        q0 = pl.multiple_of(i * _DENSE_ROWS, _DENSE_ROWS)
        s = _dot_nt(q_ref[pl.ds(q0, _DENSE_ROWS), :], k_ref[...])
        s = s.astype(dt).astype(jnp.float32) * scale
        s = s.astype(dt).astype(jnp.float32)
        rel = (
            lax.broadcasted_iota(jnp.int32, s.shape, 0)
            - lax.broadcasted_iota(jnp.int32, s.shape, 1)
            + q0
        )
        s = jnp.where((rel >= 0) & (rel < _WINDOW), s, masked)
        p = jnp.exp(s - jnp.max(s, axis=1, keepdims=True))
        o = jnp.dot(p.astype(dt), v_ref[...], preferred_element_type=jnp.float32)
        o = o / jnp.sum(p, axis=1, keepdims=True)
        o_ref[pl.ds(q0, _DENSE_ROWS), :] = o.astype(o_ref.dtype)


def _kernel(q, k, v, o, qb, kb, vb, ob, rsem, tsem, wsem):
    pairs, _, seq, dim = q.shape
    starts = [sum(_READ_CHUNKS[:i]) for i in range(len(_READ_CHUNKS))]
    last = len(_READ_CHUNKS) - 1

    def loads(ci):
        par, g0 = divmod(starts[ci], pairs)
        heads = pl.ds(g0, _READ_CHUNKS[ci])
        parts = [
            (q, qb, pl.ds(0, seq), rsem.at[0, ci]),
            (k, kb, pl.ds(0, seq), rsem.at[1, ci]),
        ]
        if ci == last:
            cut = seq - _READ_TAIL
            parts.append((v, vb, pl.ds(0, cut), rsem.at[2, ci]))
            parts.append((v, vb, pl.ds(cut, _READ_TAIL), tsem))
        else:
            parts.append((v, vb, pl.ds(0, seq), rsem.at[2, ci]))
        return [
            pltpu.make_async_copy(
                src.at[heads, par, rows], dst.at[heads, par, rows], sem
            )
            for src, dst, rows, sem in parts
        ]

    def stores(par):
        copies = []
        for j in range(seq // _WRITE_ROWS):
            rows = pl.ds(j * _WRITE_ROWS, _WRITE_ROWS)
            copies.append(
                pltpu.make_async_copy(
                    ob.at[:, par, rows], o.at[:, par, rows], wsem.at[par, j]
                )
            )
        return copies

    for ci in range(len(_READ_CHUNKS)):
        for cp in loads(ci):
            cp.start()

    safe = 0.5 * _MASK_VALUE * dim**0.5

    @pl.loop(0, 2 * pairs)
    def _(t):
        for ci in range(len(_READ_CHUNKS)):

            @pl.when(t == starts[ci])
            def _():
                copies = loads(ci)
                for cp in copies[:3]:
                    cp.wait()
                if ci == last:
                    for cp in stores(0):
                        cp.start()
                    copies[3].wait()

        par, g = t // pairs, t % pairs
        refs = [b.at[g, par] for b in (qb, kb, vb, ob)]
        low = _banded_head(*refs)

        @pl.when(jnp.logical_not(low >= safe))
        def _():
            _dense_head(*refs)

    for cp in stores(1):
        cp.start()
    for cp in stores(0) + stores(1):
        cp.wait()


@jax.jit
def pallas_standalone__sliding_local_fixed_window__prompt_kernel(
    q: jax.Array,
    k: jax.Array,
    v: jax.Array,
):
    batch, heads, seq, dim = q.shape
    assert batch * heads == sum(_READ_CHUNKS) and (seq - _TILE) % _QBLK == 0
    shape = (batch * heads // 2, 2, seq, dim)
    hbm = pl.BlockSpec(memory_space=pl.ANY)
    out = pl.pallas_call(
        _kernel,
        in_specs=[hbm, hbm, hbm],
        out_specs=hbm,
        out_shape=jax.ShapeDtypeStruct(shape, q.dtype),
        scratch_shapes=[
            pltpu.VMEM(shape, q.dtype),
            pltpu.VMEM(shape, k.dtype),
            pltpu.VMEM(shape, v.dtype),
            pltpu.VMEM(shape, q.dtype),
            pltpu.SemaphoreType.DMA((3, len(_READ_CHUNKS))),
            pltpu.SemaphoreType.DMA(()),
            pltpu.SemaphoreType.DMA((2, seq // _WRITE_ROWS)),
        ],
        compiler_params=pltpu.CompilerParams(vmem_limit_bytes=100 * 2**20),
    )(q.reshape(shape), k.reshape(shape), v.reshape(shape))
    return out.reshape(q.shape)
```

```python
import jax
import jax.numpy as jnp
import numpy as np
from jax import lax
import jax.experimental.pallas as pl
import jax.experimental.pallas.tpu as pltpu

_WINDOW = 32
_MASK_VALUE = -1e9
_TILE = 128
_QBLK = _TILE - _WINDOW
_READ_CHUNKS = (8, 8, 9, 7)
_READ_TAIL = 224
_WRITE_ROWS = 128
_DENSE_ROWS = 16


def _dot_nt(a, b):
    return lax.dot_general(
        a, b, (((1,), (1,)), ((), ())), preferred_element_type=jnp.float32
    )


def _banded_head(q_ref, k_ref, v_ref, o_ref):
    seq, dim = q_ref.shape
    c = float(dim**-0.5 * np.log2(np.e))

    def block(q0, rows, k0, mask):
        s = _dot_nt(q_ref[q0 : q0 + rows, :], k_ref[k0 : k0 + _TILE, :])
        s = jnp.where(mask, s, -jnp.inf)
        m = jnp.max(s, axis=1, keepdims=True)
        p = jnp.exp2((s - m) * c)
        l = jnp.sum(p, axis=1, keepdims=True)
        o = jnp.dot(
            p.astype(v_ref.dtype),
            v_ref[k0 : k0 + _TILE, :],
            preferred_element_type=jnp.float32,
        )
        o_ref[q0 : q0 + rows, :] = (o / l).astype(o_ref.dtype)
        return m

    def band(rows, shift):
        rel = (
            lax.broadcasted_iota(jnp.int32, (rows, _TILE), 0)
            - lax.broadcasted_iota(jnp.int32, (rows, _TILE), 1)
            + shift
        )
        return (rel >= 0) & (rel < _WINDOW)

    first = block(0, _TILE, 0, band(_TILE, 0))
    mask = band(_QBLK, _WINDOW)
    low = None
    for q0 in range(_TILE, seq, _QBLK):
        m = block(q0, _QBLK, q0 - _WINDOW, mask)
        low = m if low is None else jnp.minimum(low, m)
    return jnp.minimum(jnp.min(first), jnp.min(low))


def _dense_head(q_ref, k_ref, v_ref, o_ref):
    seq, dim = q_ref.shape
    dt = q_ref.dtype
    scale = float(np.asarray(dim**-0.5, dtype=dt))
    masked = float(np.asarray(_MASK_VALUE, dtype=dt))

    @pl.loop(0, seq // _DENSE_ROWS)
    def _(i):
        q0 = pl.multiple_of(i * _DENSE_ROWS, _DENSE_ROWS)
        s = _dot_nt(q_ref[pl.ds(q0, _DENSE_ROWS), :], k_ref[...])
        s = s.astype(dt).astype(jnp.float32) * scale
        s = s.astype(dt).astype(jnp.float32)
        rel = (
            lax.broadcasted_iota(jnp.int32, s.shape, 0)
            - lax.broadcasted_iota(jnp.int32, s.shape, 1)
            + q0
        )
        s = jnp.where((rel >= 0) & (rel < _WINDOW), s, masked)
        p = jnp.exp(s - jnp.max(s, axis=1, keepdims=True))
        o = jnp.dot(p.astype(dt), v_ref[...], preferred_element_type=jnp.float32)
        o = o / jnp.sum(p, axis=1, keepdims=True)
        o_ref[pl.ds(q0, _DENSE_ROWS), :] = o.astype(o_ref.dtype)


def _kernel(q, k, v, o, qb, kb, vb, ob, rsem, tsem, wsem):
    pairs, _, seq, dim = q.shape
    starts = [sum(_READ_CHUNKS[:i]) for i in range(len(_READ_CHUNKS))]
    last = len(_READ_CHUNKS) - 1

    def loads(ci):
        par, g0 = divmod(starts[ci], pairs)
        heads = pl.ds(g0, _READ_CHUNKS[ci])
        cut = seq - _READ_TAIL if ci == last else seq
        parts = [
            (q, qb, pl.ds(0, seq), rsem.at[ci]),
            (k, kb, pl.ds(0, seq), rsem.at[ci]),
            (v, vb, pl.ds(0, cut), rsem.at[ci]),
        ]
        if ci == last:
            parts.append((v, vb, pl.ds(cut, _READ_TAIL), tsem))
        return [
            pltpu.make_async_copy(
                src.at[heads, par, rows], dst.at[heads, par, rows], sem
            )
            for src, dst, rows, sem in parts
        ]

    def stores(par):
        copies = []
        for j in range(seq // _WRITE_ROWS):
            rows = pl.ds(j * _WRITE_ROWS, _WRITE_ROWS)
            copies.append(
                pltpu.make_async_copy(ob.at[:, par, rows], o.at[:, par, rows], wsem)
            )
        return copies

    for ci in range(len(_READ_CHUNKS)):
        for cp in loads(ci):
            cp.start()

    safe = 0.5 * _MASK_VALUE * dim**0.5

    @pl.loop(0, 2 * pairs)
    def _(t):
        for ci in range(len(_READ_CHUNKS)):

            @pl.when(t == starts[ci])
            def _():
                copies = loads(ci)
                for cp in copies[:3]:
                    cp.wait()
                if ci == last:
                    for cp in stores(0):
                        cp.start()
                    copies[3].wait()

        par, g = t // pairs, t % pairs
        refs = [b.at[g, par] for b in (qb, kb, vb, ob)]
        low = _banded_head(*refs)

        @pl.when(jnp.logical_not(low >= safe))
        def _():
            _dense_head(*refs)

    for cp in stores(1):
        cp.start()
    for cp in stores(0) + stores(1):
        cp.wait()


@jax.jit
def pallas_standalone__sliding_local_fixed_window__prompt_kernel(
    q: jax.Array,
    k: jax.Array,
    v: jax.Array,
):
    batch, heads, seq, dim = q.shape
    assert batch * heads == sum(_READ_CHUNKS) and (seq - _TILE) % _QBLK == 0
    shape = (batch * heads // 2, 2, seq, dim)
    hbm = pl.BlockSpec(memory_space=pl.ANY)
    out = pl.pallas_call(
        _kernel,
        in_specs=[hbm, hbm, hbm],
        out_specs=hbm,
        out_shape=jax.ShapeDtypeStruct(shape, q.dtype),
        scratch_shapes=[
            pltpu.VMEM(shape, q.dtype),
            pltpu.VMEM(shape, k.dtype),
            pltpu.VMEM(shape, v.dtype),
            pltpu.VMEM(shape, q.dtype),
            pltpu.SemaphoreType.DMA((len(_READ_CHUNKS),)),
            pltpu.SemaphoreType.DMA(()),
            pltpu.SemaphoreType.DMA(()),
        ],
        compiler_params=pltpu.CompilerParams(vmem_limit_bytes=100 * 2**20),
    )(q.reshape(shape), k.reshape(shape), v.reshape(shape))
    return out.reshape(q.shape)
```
